```python
import jax
import jax.numpy as jnp

def _softmax(x, axis=-1):
    return jax.nn.softmax(x, axis=axis)
def _gelu(x):
    return jax.nn.gelu(x, approximate=True)
def _silu(x):
    return jax.nn.silu(x)
def _sigmoid(x):
    return jax.nn.sigmoid(x)
def _layernorm(x, axis=-1, eps=1e-5):
    m = jnp.mean(x, axis=axis, keepdims=True)
    v = jnp.var(x, axis=axis, keepdims=True)
    return (x - m) / jnp.sqrt(v + eps)
def _scatter_add(tgt, idx, src, axis=0):
    return tgt.at[idx].add(src)
def _segment_sum(src, seg, n):
    return jax.ops.segment_sum(src, seg, n)
class _Rng:
    def __init__(self, key):
        self._k = key
    def _next(self):
        self._k, sub = jax.random.split(self._k)
        return sub
    def normal(self, shape):
        return jax.random.normal(self._next(), shape, dtype=jnp.bfloat16)
    def randint(self, lo, hi, shape):
        return jax.random.randint(self._next(), shape, lo, hi, dtype=jnp.int32)
    def uniform(self, shape, lo=0.0, hi=1.0):
        return jax.random.uniform(self._next(), shape, jnp.bfloat16, lo, hi)
    def permutation(self, n):
        return jax.random.permutation(self._next(), n)


kernel_name = 'standalone__winograd__vision'

def setup_inputs():
    _rng = _Rng(jax.random.key(int.from_bytes(__import__("os").urandom(4), "little")))
    _w = (lambda a: (lambda t: t.astype(jnp.bfloat16) if jnp.issubdtype(t.dtype, jnp.floating) else t)(jnp.asarray(a)))
    H = W = 512 // 2 * 2
    C = 192
    return {
        "x": _w((lambda *s: _rng.normal(s) * 0.05)(1, H, W, C)),
        "w": _w((lambda *s: _rng.normal(s) * 0.05)(3, 3, C, C)),
    }

def reference(x, w):
    N, H, W, C = x.shape
    K = w.shape[-1]
    G  = jnp.array([[1.0,0.0,0.0],[0.5,0.5,0.5],[0.5,-0.5,0.5],[0.0,0.0,1.0]], dtype=x.dtype)
    Bt = jnp.array([[1.0,0.0,-1.0,0.0],[0.0,1.0,1.0,0.0],[0.0,-1.0,1.0,0.0],[0.0,1.0,0.0,-1.0]], dtype=x.dtype)
    At = jnp.array([[1.0,1.0,1.0,0.0],[0.0,1.0,-1.0,-1.0]], dtype=x.dtype)
    U = jnp.einsum("ar,rsck,bs->abck", G, w, G)
    xp = jnp.pad(x, ((0,0),(1,1),(1,1),(0,0)))
    nH, nW = H // 2, W // 2
    patches = []
    for i in range(4):
        for j in range(4):
            patches.append(xp[:, i:i + 2 * nH:2, j:j + 2 * nW:2, :])
    d = jnp.stack(patches).reshape(4, 4, N * nH * nW, C)
    V = jnp.einsum("ai,ijpc,bj->abpc", Bt, d, Bt)
    M = jnp.einsum("abck,abpc->abpk", U, V)
    Y = jnp.einsum("ma,abpk,nb->pmnk", At, M, At)
    Y = Y.reshape(N, nH, nW, 2, 2, K)
    Y = (lambda x, *d: x.transpose(*d))(Y, 0, 1, 3, 2, 4, 5).reshape(N, H, W, K)
    return Y
```

```python
import numpy as np
import jax
import jax.numpy as jnp
from jax import lax
import jax.experimental.pallas as pl
import jax.experimental.pallas.tpu as pltpu


def _toom_cook(m, pts):
    n = m + 2
    at, g, bt = np.zeros((m, n)), np.zeros((n, 3)), np.zeros((n, n))
    for i, p in enumerate(pts):
        others = [q for j, q in enumerate(pts) if j != i]
        f = float(np.prod([p - q for q in others]))
        at[:, i] = [float(p) ** k for k in range(m)]
        g[i] = [float(p) ** k / f for k in range(3)]
        co = np.poly(others)[::-1]
        bt[i, :len(co)] = co
    at[m - 1, n - 1] = 1.0
    g[n - 1, 2] = 1.0
    bt[n - 1] = np.poly(pts)[::-1]
    return at, g, bt


M_ = 4
AT, G_, BT = _toom_cook(M_, {2: [0, 1, -1], 4: [0, 1, -1, .5, -2]}[M_])
NA = M_ + 2
GROUPS = 4
R = M_ * GROUPS
CH = 32
NB = 512


def _lin(coefs, vals):
    acc = None
    for c, v in zip(coefs, vals):
        c = float(c)
        if c == 0:
            continue
        t = v if abs(c) == 1 else v * abs(c)
        if acc is None:
            acc = t if c > 0 else -t
        else:
            acc = acc + t if c > 0 else acc - t
    return acc


def _kernel(xm, xp, xn, w_ref, o_ref, u_ref, v_ref, *, C, K, W):
    i = pl.program_id(0)
    last = pl.num_programs(0) - 1

    @pl.when(i == 0)
    def _():
        ws = [w_ref[r].astype(jnp.float32) for r in range(3)]
        for a in range(NA):
            u_ref[a] = _lin(G_[a], ws).astype(jnp.bfloat16)

    lane = lax.broadcasted_iota(jnp.int32, (CH // 2, W), 1)

    def row(h, cs):
        if h < 0:
            t = xp[0, cs, :]
            return jnp.where(i > 0, t, jnp.zeros_like(t)).astype(jnp.float32)
        if h >= R:
            t = xn[0, cs, :]
            return jnp.where(i < last, t, jnp.zeros_like(t)).astype(jnp.float32)
        return xm[h, cs, :].astype(jnp.float32)

    def transform(g):
        for c in range(0, C, CH):
            d = [row(g * M_ - 1 + r, pl.ds(c, CH)) for r in range(NA)]
            for a in range(NA):
                v = pltpu.bitcast(_lin(BT[a], d).astype(jnp.bfloat16), jnp.uint32)
                lft = jnp.where(lane == 0, jnp.uint32(0), pltpu.roll(v, 1, 1))
                rgt = jnp.where(lane == W - 1, jnp.uint32(0), pltpu.roll(v, W - 1, 1))
                for s, t in enumerate((lft, v, rgt)):
                    v_ref[g % 2, a, pl.ds(s * C + c, CH), :] = pltpu.bitcast(t, jnp.bfloat16)

    def matmul(g):
        for n in range(0, W, NB):
            ms = [jnp.dot(u_ref[a], v_ref[g % 2, a, :, pl.ds(n, NB)],
                          preferred_element_type=jnp.float32) for a in range(NA)]
            for r in range(M_):
                o_ref[g * M_ + r, :, pl.ds(n, NB)] = _lin(AT[r], ms).astype(o_ref.dtype)

    transform(0)
    for g in range(GROUPS):
        if g + 1 < GROUPS:
            transform(g + 1)
        matmul(g)


@jax.jit
def pallas_standalone__winograd__vision_kernel(x: jax.Array, w: jax.Array):
    N, H, W, C = x.shape
    K = w.shape[-1]
    assert N == 1 and H % R == 0
    xt = x.transpose(0, 1, 3, 2).reshape(H, C, W)
    wt = w.transpose(0, 3, 1, 2).reshape(3, K, 3 * C)
    nb = H // R
    import functools
    out = pl.pallas_call(
        functools.partial(_kernel, C=C, K=K, W=W),
        grid=(nb,),
        in_specs=[
            pl.BlockSpec((R, C, W), lambda i: (i, 0, 0)),
            pl.BlockSpec((1, C, W), lambda i: (jnp.maximum(i * R - 1, 0), 0, 0)),
            pl.BlockSpec((1, C, W), lambda i: (jnp.minimum(i * R + R, H - 1), 0, 0)),
            pl.BlockSpec((3, K, 3 * C), lambda i: (0, 0, 0)),
        ],
        out_specs=pl.BlockSpec((R, K, W), lambda i: (i, 0, 0)),
        out_shape=jax.ShapeDtypeStruct((H, K, W), x.dtype),
        scratch_shapes=[pltpu.VMEM((NA, K, 3 * C), jnp.bfloat16),
                        pltpu.VMEM((2, NA, 3 * C, W), jnp.bfloat16)],
        compiler_params=pltpu.CompilerParams(
            dimension_semantics=("arbitrary",), vmem_limit_bytes=100 * 2**20),
    )(xt, xt, xt, wt)
    return out.reshape(N, H, K, W).transpose(0, 1, 3, 2)
```

```python
import numpy as np
import jax
import jax.numpy as jnp
from jax import lax
import jax.experimental.pallas as pl
import jax.experimental.pallas.tpu as pltpu


def _toom_cook(m, pts):
    n = m + 2
    at, g, bt = np.zeros((m, n)), np.zeros((n, 3)), np.zeros((n, n))
    for i, p in enumerate(pts):
        others = [q for j, q in enumerate(pts) if j != i]
        f = float(np.prod([p - q for q in others]))
        at[:, i] = [float(p) ** k for k in range(m)]
        g[i] = [float(p) ** k / f for k in range(3)]
        co = np.poly(others)[::-1]
        bt[i, :len(co)] = co
    at[m - 1, n - 1] = 1.0
    g[n - 1, 2] = 1.0
    bt[n - 1] = np.poly(pts)[::-1]
    return at, g, bt


M_ = 4
AT, G_, BT = _toom_cook(M_, {2: [0, 1, -1], 4: [0, 1, -1, .5, -2]}[M_])
NA = M_ + 2
GROUPS = 4
R = M_ * GROUPS
CH = 32
NB = 512


def _lin(coefs, vals):
    acc = None
    for c, v in zip(coefs, vals):
        c = float(c)
        if c == 0:
            continue
        t = v if abs(c) == 1 else v * abs(c)
        if acc is None:
            acc = t if c > 0 else -t
        else:
            acc = acc + t if c > 0 else acc - t
    return acc


def _kernel(xm, xn, w_ref, o_ref, u_ref, v_ref, *, C, K, W):
    i = pl.program_id(0)
    last = pl.num_programs(0) - 1

    @pl.when(i == 0)
    def _():
        ws = [w_ref[r].astype(jnp.float32) for r in range(3)]
        for a in range(NA):
            u_ref[a] = pltpu.bitcast(_lin(G_[a], ws).astype(jnp.bfloat16), jnp.uint32)

    lane = lax.broadcasted_iota(jnp.int32, (CH // 2, W), 1)

    def row(h, cs):
        if h < 0:
            return jnp.zeros((CH, W), jnp.float32)
        if h >= R:
            t = xn[h - R, cs, :]
            if h > R:
                return t.astype(jnp.float32)
            return jnp.where(i < last, t, jnp.zeros_like(t)).astype(jnp.float32)
        return xm[h, cs, :].astype(jnp.float32)

    def transform(g):
        for c in range(0, C, CH):
            d = [row(g * M_ - 1 + r, pl.ds(c, CH)) for r in range(NA)]
            for a in range(NA):
                v = pltpu.bitcast(_lin(BT[a], d).astype(jnp.bfloat16), jnp.uint32)
                lft = jnp.where(lane == 0, jnp.uint32(0), pltpu.roll(v, 1, 1))
                rgt = jnp.where(lane == W - 1, jnp.uint32(0), pltpu.roll(v, W - 1, 1))
                for s, t in enumerate((lft, v, rgt)):
                    v_ref[g % 2, a, pl.ds((s * C + c) // 2, CH // 2), :] = t

    def matmul(g):
        for n in range(0, W, NB):
            ms = [jnp.dot(pltpu.bitcast(u_ref[a], jnp.bfloat16),
                          pltpu.bitcast(v_ref[g % 2, a, :, pl.ds(n, NB)], jnp.bfloat16),
                          preferred_element_type=jnp.float32) for a in range(NA)]
            for r in range(M_):
                o_ref[g * M_ + r, :, pl.ds(n, NB)] = _lin(AT[r], ms).astype(o_ref.dtype)

    @pl.when(i == 0)
    def _():
        transform(0)

    for g in range(GROUPS):
        transform(g + 1)
        matmul(g)


@jax.jit
def pallas_standalone__winograd__vision_kernel(x: jax.Array, w: jax.Array):
    N, H, W, C = x.shape
    K = w.shape[-1]
    assert N == 1 and H % R == 0
    xt = x.transpose(0, 1, 3, 2).reshape(H, C, W)
    wt = w.transpose(0, 3, 1, 2).reshape(3, K, 3 * C)
    nb = H // R
    import functools
    out = pl.pallas_call(
        functools.partial(_kernel, C=C, K=K, W=W),
        grid=(nb,),
        in_specs=[
            pl.BlockSpec((R, C, W), lambda i: (i, 0, 0)),
            pl.BlockSpec((8, C, W), lambda i: (jnp.minimum((i + 1) * (R // 8), H // 8 - 1), 0, 0)),
            pl.BlockSpec((3, K, 3 * C), lambda i: (0, 0, 0)),
        ],
        out_specs=pl.BlockSpec((R, K, W), lambda i: (i, 0, 0)),
        out_shape=jax.ShapeDtypeStruct((H, K, W), x.dtype),
        scratch_shapes=[pltpu.VMEM((NA, K // 2, 3 * C), jnp.uint32),
                        pltpu.VMEM((2, NA, 3 * C // 2, W), jnp.uint32)],
        compiler_params=pltpu.CompilerParams(
            dimension_semantics=("arbitrary",), vmem_limit_bytes=100 * 2**20),
    )(xt, xt, wt)
    return out.reshape(N, H, K, W).transpose(0, 1, 3, 2)
```

```python
import numpy as np
import jax
import jax.numpy as jnp
from jax import lax
import jax.experimental.pallas as pl
import jax.experimental.pallas.tpu as pltpu


def _toom_cook(m, pts):
    n = m + 2
    at, g, bt = np.zeros((m, n)), np.zeros((n, 3)), np.zeros((n, n))
    for i, p in enumerate(pts):
        others = [q for j, q in enumerate(pts) if j != i]
        f = float(np.prod([p - q for q in others]))
        at[:, i] = [float(p) ** k for k in range(m)]
        g[i] = [float(p) ** k / f for k in range(3)]
        co = np.poly(others)[::-1]
        bt[i, :len(co)] = co
    at[m - 1, n - 1] = 1.0
    g[n - 1, 2] = 1.0
    bt[n - 1] = np.poly(pts)[::-1]
    return at, g, bt


M_ = 6
AT, G_, BT = _toom_cook(M_, {2: [0, 1, -1], 6: [0, 1, -1, .5, -.5, 2, -2], 4: [0, 1, -1, .5, -2]}[M_])
NA = M_ + 2
GROUPS = 2
R = M_ * GROUPS
CH = 32
NB = 512


def _lin(coefs, vals):
    acc = None
    for c, v in zip(coefs, vals):
        c = float(c)
        if abs(c) < 1e-9:
            continue
        t = v if abs(c) == 1 else v * abs(c)
        if acc is None:
            acc = t if c > 0 else -t
        else:
            acc = acc + t if c > 0 else acc - t
    return acc


def _kernel(xm, xn, w_ref, o_ref, u_ref, v_ref, *, C, K, W, H):
    i = pl.program_id(0)
    last = pl.num_programs(0) - 1

    @pl.when(i == 0)
    def _():
        ws = [w_ref[r].astype(jnp.float32) for r in range(3)]
        for a in range(NA):
            u_ref[a] = pltpu.bitcast(_lin(G_[a], ws).astype(jnp.bfloat16), jnp.uint32)

    lane = lax.broadcasted_iota(jnp.int32, (CH // 2, W), 1)

    def row(h, cs):
        if h < 0:
            return jnp.zeros((CH, W), jnp.float32)
        if h >= R:
            t = xn[h - R, cs, :]
            return jnp.where(i * R + h < H, t, jnp.zeros_like(t)).astype(jnp.float32)
        t = xm[h, cs, :]
        if h >= H - (H - 1) // R * R:
            t = jnp.where(i * R + h < H, t, jnp.zeros_like(t))
        return t.astype(jnp.float32)

    def transform(g):
        for c in range(0, C, CH):
            d = [row(g * M_ - 1 + r, pl.ds(c, CH)) for r in range(NA)]
            vs = [_lin(BT[0], d)]
            for j in (1, 3, 5):
                ev = _lin((BT[j] + BT[j + 1]) / 2, d)
                od = _lin((BT[j] - BT[j + 1]) / 2, d)
                vs += [ev + od, ev - od]
            vs.append(_lin(BT[7], d))
            for a in range(NA):
                v = pltpu.bitcast(vs[a].astype(jnp.bfloat16), jnp.uint32)
                lft = jnp.where(lane == 0, jnp.uint32(0), pltpu.roll(v, 1, 1))
                rgt = jnp.where(lane == W - 1, jnp.uint32(0), pltpu.roll(v, W - 1, 1))
                for s, t in enumerate((lft, v, rgt)):
                    v_ref[g % 2, a, pl.ds((s * C + c) // 2, CH // 2), :] = t

    def matmul(g):
        for n in range(0, W, NB):
            ms = [jnp.dot(pltpu.bitcast(u_ref[a], jnp.bfloat16),
                          pltpu.bitcast(v_ref[g % 2, a, :, pl.ds(n, NB)], jnp.bfloat16),
                          preferred_element_type=jnp.float32) for a in range(NA)]
            sm = [ms[j] + ms[j + 1] for j in (1, 3, 5)]
            df = [ms[j] - ms[j + 1] for j in (1, 3, 5)]
            for r in range(M_):
                y = _lin(AT[r, 1:7:2], df if r % 2 else sm)
                if r == 0:
                    y = y + ms[0]
                if r == M_ - 1:
                    y = y + ms[7]
                o_ref[g * M_ + r, :, pl.ds(n, NB)] = y.astype(o_ref.dtype)

    @pl.when(i == 0)
    def _():
        transform(0)

    for g in range(GROUPS):
        transform(g + 1)
        matmul(g)


@jax.jit
def pallas_standalone__winograd__vision_kernel(x: jax.Array, w: jax.Array):
    N, H, W, C = x.shape
    K = w.shape[-1]
    assert N == 1 and R == 12 and H % 2 == 0
    xt = x.transpose(0, 1, 3, 2).reshape(H, C, W)
    wt = w.transpose(0, 3, 1, 2).reshape(3, K, 3 * C)
    nb = pl.cdiv(H, R)
    import functools
    out = pl.pallas_call(
        functools.partial(_kernel, C=C, K=K, W=W, H=H),
        grid=(nb,),
        in_specs=[
            pl.BlockSpec((R, C, W), lambda i: (i, 0, 0)),
            pl.BlockSpec((R, C, W), lambda i: (jnp.minimum(i + 1, nb - 1), 0, 0)),
            pl.BlockSpec((3, K, 3 * C), lambda i: (0, 0, 0)),
        ],
        out_specs=pl.BlockSpec((R, K, W), lambda i: (i, 0, 0)),
        out_shape=jax.ShapeDtypeStruct((H, K, W), x.dtype),
        scratch_shapes=[pltpu.VMEM((NA, K // 2, 3 * C), jnp.uint32),
                        pltpu.VMEM((2, NA, 3 * C // 2, W), jnp.uint32)],
        compiler_params=pltpu.CompilerParams(
            dimension_semantics=("arbitrary",), vmem_limit_bytes=100 * 2**20),
    )(xt, xt, wt)
    return out.reshape(N, H, K, W).transpose(0, 1, 3, 2)
```
